```python
import os as _os
_os.environ.setdefault("JAX_PLATFORMS", "cpu")
import jax
import jax.numpy as jnp

def _softmax(x, axis=-1):
    return jax.nn.softmax(x, axis=axis)
def _gelu(x):
    return jax.nn.gelu(x, approximate=True)
def _silu(x):
    return jax.nn.silu(x)
def _sigmoid(x):
    return jax.nn.sigmoid(x)
def _layernorm(x, axis=-1, eps=1e-5):
    m = jnp.mean(x, axis=axis, keepdims=True)
    v = jnp.var(x, axis=axis, keepdims=True)
    return (x - m) / jnp.sqrt(v + eps)
def _scatter_add(tgt, idx, src, axis=0):
    return tgt.at[idx].add(src)
def _segment_sum(src, seg, n):
    return jax.ops.segment_sum(src, seg, n)
class _Rng:
    def __init__(self, key):
        self._k = key
    def _next(self):
        self._k, sub = jax.random.split(self._k)
        return sub
    def normal(self, shape):
        return jax.random.normal(self._next(), shape, dtype=jnp.bfloat16)
    def randint(self, lo, hi, shape):
        return jax.random.randint(self._next(), shape, lo, hi, dtype=jnp.int32)
    def uniform(self, shape, lo=0.0, hi=1.0):
        return jax.random.uniform(self._next(), shape, jnp.bfloat16, lo, hi)
    def permutation(self, n):
        return jax.random.permutation(self._next(), n)


kernel_name = 'gated_mix__mha_block__mha_block__prompt'

def setup_inputs():
    _rng = _Rng(jax.random.key(int.from_bytes(__import__("os").urandom(4), "little")))
    _w = (lambda a: (lambda t: t.astype(jnp.bfloat16) if jnp.issubdtype(t.dtype, jnp.floating) else t)(jnp.asarray(a)))
    def _A_setup():
        B, S, D, H = 1, 2048, 448, 16
        return {
            "x": _w((lambda *s: _rng.normal(s) * 0.05)(B, S, D)),
            "wqkv": _w((lambda *s: _rng.normal(s) * 0.4)(D, 3 * D)),
            "wo": _w((lambda *s: _rng.normal(s) * 0.05)(D, D)),
        }
    _A_in = _A_setup()

    def _B_setup():
        B, S, D, H = 1, 2048, 448, 16
        return {
            "x": _w((lambda *s: _rng.normal(s) * 0.05)(B, S, D)),
            "wqkv": _w((lambda *s: _rng.normal(s) * 0.4)(D, 3 * D)),
            "wo": _w((lambda *s: _rng.normal(s) * 0.05)(D, D)),
        }
    _B_in = _B_setup()

    return {
        "A_x": _A_in["x"],
        "A_wqkv": _A_in["wqkv"],
        "A_wo": _A_in["wo"],
        "B_x": _B_in["x"],
        "B_wqkv": _B_in["wqkv"],
        "B_wo": _B_in["wo"],
        "gate_w": _w((lambda *s: _rng.normal(s) * 0.05)(448) * 16.0),
    }

def reference(A_x, A_wqkv, A_wo, B_x, B_wqkv, B_wo, gate_w):
    def _A_ref(x, wqkv, wo):
        B, S, D = x.shape
        H = 16
        Dh = D // H
        qkv = (lambda x, *d: x.transpose(*d))((x @ wqkv).reshape(B, S, 3, H, Dh), 2, 0, 3, 1, 4)
        q, k, v = qkv[0], qkv[1], qkv[2]
        scores = jnp.einsum("bhqd,bhkd->bhqk", q, k) * (Dh ** -0.5)
        p = _softmax(scores, axis=-1)
        o = jnp.einsum("bhqk,bhkd->bhqd", p, v)
        return (lambda x, *d: x.transpose(*d))(o, 0, 2, 1, 3).reshape(B, S, D) @ wo

    def _B_ref(x, wqkv, wo):
        B, S, D = x.shape
        H = 16
        Dh = D // H
        qkv = (lambda x, *d: x.transpose(*d))((x @ wqkv).reshape(B, S, 3, H, Dh), 2, 0, 3, 1, 4)
        q, k, v = qkv[0], qkv[1], qkv[2]
        scores = jnp.einsum("bhqd,bhkd->bhqk", q, k) * (Dh ** -0.5)
        p = _softmax(scores, axis=-1)
        o = jnp.einsum("bhqk,bhkd->bhqd", p, v)
        return (lambda x, *d: x.transpose(*d))(o, 0, 2, 1, 3).reshape(B, S, D) @ wo

    x = A_x
    g = _sigmoid((x * gate_w).sum(-1, keepdims=True))
    a = _A_ref(x, A_wqkv, A_wo)
    b = _B_ref(x, B_wqkv, B_wo)
    return g * a + (1 - g) * b
```

```python
import functools, math
import jax, jax.numpy as jnp
from jax import lax
from jax.experimental import pallas as pl
from jax.experimental.pallas import tpu as pltpu

S, D, H, DH, DP = 2048, 448, 16, 28, 32
NH = 2 * H
HP = H * DP
QSCALE = (DH ** -0.5) * math.log2(math.e)

def _make(TQ=512):
    NQ = S // TQ
    def kernel(x_ref, wqvt_ref, wk_ref, wot_ref, o_ref, qvt_s, kh_s, ot_s, g_s):
        x = x_ref[...]
        NT = (((1,), (1,)), ((), ()))
        for r in range(4):
            t = lax.dot_general(wqvt_ref[r * HP:(r + 1) * HP, :], x, NT, preferred_element_type=jnp.float32)
            if r % 2 == 0:
                t = t * QSCALE
            else:
                row = lax.broadcasted_iota(jnp.int32, (HP, 1), 0)
                t = jnp.where(row % DP == DH, 1.0, t)
            qvt_s[r * HP:(r + 1) * HP, :] = t.astype(jnp.bfloat16)
        gl = lax.dot_general(wqvt_ref[4 * HP:4 * HP + 16, :], x, NT, preferred_element_type=jnp.float32)
        g_s[...] = jax.nn.sigmoid(gl[0:8, :])
        for grp in range(8):
            kk = jnp.dot(x, wk_ref[:, grp * 128:(grp + 1) * 128], preferred_element_type=jnp.float32)
            for j in range(4):
                kh_s[grp * 4 + j] = kk[:, j * DP:(j + 1) * DP].astype(jnp.bfloat16)

        def head_body(h, carry):
            br = h // H
            hh = h % H
            qrow = pl.multiple_of(br * 2 * HP + hh * DP, DP)
            vrow = pl.multiple_of(br * 2 * HP + HP + hh * DP, DP)
            kh = kh_s[h]
            vt = qvt_s[pl.ds(vrow, DP), :]
            for qi in range(NQ):
                qt = qvt_s[pl.ds(qrow, DP), qi * TQ:(qi + 1) * TQ]
                st = jnp.dot(kh, qt, preferred_element_type=jnp.float32)
                m = jnp.max(st, axis=0, keepdims=True)
                p = jnp.exp2(st - m).astype(jnp.bfloat16)
                ot = jnp.dot(vt, p, preferred_element_type=jnp.float32)
                l = ot[DH:DH + 1, :]
                g = g_s[0:1, qi * TQ:(qi + 1) * TQ]
                gg = jnp.where(br == 0, g, 1.0 - g)
                ot = ot * (gg / l)
                ot_s[pl.ds(pl.multiple_of(h * DP, DP), DP), qi * TQ:(qi + 1) * TQ] = ot.astype(jnp.bfloat16)
            return carry
        lax.fori_loop(0, NH, head_body, 0)

        outt = jnp.dot(wot_ref[...], ot_s[...], preferred_element_type=jnp.float32)
        o_ref[...] = outt.T.astype(o_ref.dtype)

    @jax.jit
    def f(A_x, A_wqkv, A_wo, B_x, B_wqkv, B_wo, gate_w):
        x = A_x.reshape(S, D)
        def prep(w):
            w = jnp.pad(w.reshape(D, 3, H, DH), ((0, 0), (0, 0), (0, 0), (0, DP - DH))).reshape(D, 3, HP)
            return w[:, 0], w[:, 1], w[:, 2]
        qa, ka, va = prep(A_wqkv)
        qb, kb, vb = prep(B_wqkv)
        gpad = jnp.pad(gate_w.reshape(D, 1), ((0, 0), (0, 15)))
        wqvt = jnp.concatenate([qa, va, qb, vb, gpad], axis=1).T
        wk = jnp.concatenate([ka, kb], axis=1)
        def prepo(w):
            return jnp.pad(w.reshape(H, DH, D), ((0, 0), (0, DP - DH), (0, 0))).reshape(HP, D)
        wot = jnp.concatenate([prepo(A_wo), prepo(B_wo)], axis=0).T
        out = pl.pallas_call(
            kernel,
            out_shape=jax.ShapeDtypeStruct((S, D), jnp.bfloat16),
            scratch_shapes=[
                pltpu.VMEM((4 * HP, S), jnp.bfloat16),
                pltpu.VMEM((NH, S, DP), jnp.bfloat16),
                pltpu.VMEM((NH * DP, S), jnp.bfloat16),
                pltpu.VMEM((8, S), jnp.float32),
            ],
            compiler_params=pltpu.CompilerParams(vmem_limit_bytes=100 * 2**20),
        )(x, wqvt, wk, wot)
        return out.reshape(1, S, D)
    return f


pallas_gated_mix__mha_block__mha_block__prompt_kernel = _make()
```

```python
import functools, math
import jax, jax.numpy as jnp
from jax import lax
from jax.experimental import pallas as pl
from jax.experimental.pallas import tpu as pltpu

S, D, H, DH, DP = 2048, 448, 16, 28, 32
NH = 2 * H
HP = H * DP
QSCALE = (DH ** -0.5) * math.log2(math.e)

def _make(TQ=1024, CK=128, look=1, do_proj=True, do_attn=True, do_out=True):
    NQ = S // TQ
    NC = S // CK
    def kernel(x_ref, wqvt_ref, wk_ref, wot_ref, o_ref, qvt_s, kh_s, ot_s, g_s):
        x = x_ref[...]
        NT = (((1,), (1,)), ((), ()))
        if do_proj:
            for r in range(4):
                t = lax.dot_general(wqvt_ref[r * HP:(r + 1) * HP, :], x, NT, preferred_element_type=jnp.float32)
                if r % 2 == 0:
                    t = t * QSCALE
                else:
                    row = lax.broadcasted_iota(jnp.int32, (HP, 1), 0)
                    t = jnp.where(row % DP == DH, 1.0, t)
                qvt_s[r * HP:(r + 1) * HP, :] = t.astype(jnp.bfloat16)
            gl = lax.dot_general(wqvt_ref[4 * HP:4 * HP + 16, :], x, NT, preferred_element_type=jnp.float32)
            g_s[...] = jax.nn.sigmoid(gl[0:8, :])
            for grp in range(8):
                kk = jnp.dot(x, wk_ref[:, grp * 128:(grp + 1) * 128], preferred_element_type=jnp.float32)
                for j in range(4):
                    kh_s[grp * 4 + j] = kk[:, j * DP:(j + 1) * DP].astype(jnp.bfloat16)

        def head_body(h, carry):
            br = h // H
            hh = h % H
            qrow = pl.multiple_of(br * 2 * HP + hh * DP, DP)
            vrow = pl.multiple_of(br * 2 * HP + HP + hh * DP, DP)
            orow = pl.multiple_of(h * DP, DP)
            steps = [(qi, c) for qi in range(NQ) for c in range(NC)]
            def scores(qi, c):
                qt = qvt_s[pl.ds(qrow, DP), qi * TQ:(qi + 1) * TQ]
                return jnp.dot(kh_s[h, c * CK:(c + 1) * CK, :], qt, preferred_element_type=jnp.float32)
            pend = [scores(*steps[j]) for j in range(look)]
            for i, (qi, c) in enumerate(steps):
                s = pend.pop(0)
                if i + look < len(steps):
                    pend.append(scores(*steps[i + look]))
                cm = jnp.max(jnp.max(s.reshape(CK // 8, 8, TQ), axis=0), axis=0, keepdims=True)
                vt = qvt_s[pl.ds(vrow, DP), c * CK:(c + 1) * CK]
                if c == 0:
                    m = cm
                    p = jnp.exp2(s - m).astype(jnp.bfloat16)
                    acc = jnp.dot(vt, p, preferred_element_type=jnp.float32)
                else:
                    mn = jnp.maximum(m, cm)
                    alpha = jnp.exp2(m - mn)
                    p = jnp.exp2(s - mn).astype(jnp.bfloat16)
                    acc = acc * alpha + jnp.dot(vt, p, preferred_element_type=jnp.float32)
                    m = mn
                if c == NC - 1:
                    l = acc[DH:DH + 1, :]
                    g = g_s[0:1, qi * TQ:(qi + 1) * TQ]
                    gg = jnp.where(br == 0, g, 1.0 - g)
                    ot_s[pl.ds(orow, DP), qi * TQ:(qi + 1) * TQ] = (acc * (gg / l)).astype(jnp.bfloat16)
            return carry
        if do_attn:
            lax.fori_loop(0, NH, head_body, 0)

        if do_out:
            outt = jnp.dot(wot_ref[...], ot_s[...], preferred_element_type=jnp.float32)
            o_ref[...] = outt.T.astype(o_ref.dtype)
        else:
            o_ref[...] = jnp.zeros(o_ref.shape, o_ref.dtype)

    @jax.jit
    def f(A_x, A_wqkv, A_wo, B_x, B_wqkv, B_wo, gate_w):
        x = A_x.reshape(S, D)
        def prep(w):
            w = jnp.pad(w.reshape(D, 3, H, DH), ((0, 0), (0, 0), (0, 0), (0, DP - DH))).reshape(D, 3, HP)
            return w[:, 0], w[:, 1], w[:, 2]
        qa, ka, va = prep(A_wqkv)
        qb, kb, vb = prep(B_wqkv)
        gpad = jnp.pad(gate_w.reshape(D, 1), ((0, 0), (0, 15)))
        wqvt = jnp.concatenate([qa, va, qb, vb, gpad], axis=1).T
        wk = jnp.concatenate([ka, kb], axis=1)
        def prepo(w):
            return jnp.pad(w.reshape(H, DH, D), ((0, 0), (0, DP - DH), (0, 0))).reshape(HP, D)
        wot = jnp.concatenate([prepo(A_wo), prepo(B_wo)], axis=0).T
        out = pl.pallas_call(
            kernel,
            out_shape=jax.ShapeDtypeStruct((S, D), jnp.bfloat16),
            scratch_shapes=[
                pltpu.VMEM((4 * HP, S), jnp.bfloat16),
                pltpu.VMEM((NH, S, DP), jnp.bfloat16),
                pltpu.VMEM((NH * DP, S), jnp.bfloat16),
                pltpu.VMEM((8, S), jnp.float32),
            ],
            compiler_params=pltpu.CompilerParams(vmem_limit_bytes=100 * 2**20),
        )(x, wqvt, wk, wot)
        return out.reshape(1, S, D)
    return f


pallas_gated_mix__mha_block__mha_block__prompt_kernel = _make()
```

```python
import functools, math
import jax, jax.numpy as jnp
from jax import lax
from jax.experimental import pallas as pl
from jax.experimental.pallas import tpu as pltpu

S, D, H, DH, DP = 2048, 448, 16, 28, 32
NH = 2 * H
HP = H * DP
QSCALE = (DH ** -0.5) * math.log2(math.e)
F32 = jnp.float32
BF16 = jnp.bfloat16

def _make(TQ=1024, CK=128, hpi=2, OC=512, do_proj=True, do_attn=True, do_out=True):
    NQ = S // TQ
    NC = S // CK
    NOC = S // OC
    def kernel(xt_hbm, wa_hbm, woa_hbm, wb_hbm, wob_hbm, gw_ref, o_hbm,
               xt_s, w_s, wo_s, wt_s, wkp_s, wop_s, tmp_s, qvt_s, kh_s, ot_s, g_s, sc_s, out_s, sems):
        NT = (((1,), (1,)), ((), ()))
        cp_wa = pltpu.make_async_copy(wa_hbm, w_s.at[0], sems.at[0])
        cp_x = pltpu.make_async_copy(xt_hbm, xt_s, sems.at[1])
        cp_wb = pltpu.make_async_copy(wb_hbm, w_s.at[1], sems.at[2])
        cp_woa = pltpu.make_async_copy(woa_hbm, wo_s.at[0], sems.at[3])
        cp_wob = pltpu.make_async_copy(wob_hbm, wo_s.at[1], sems.at[4])
        for cp in (cp_wa, cp_x, cp_wb, cp_woa, cp_wob):
            cp.start()
        zpad = jnp.zeros((DP - DH, D), F32)
        zrow = jnp.zeros((DP - DH, S), F32)
        prow = lax.broadcasted_iota(jnp.int32, (DP - DH, S), 0)
        onerow = jnp.where(prow == 0, 1.0, 0.0).astype(F32)
        grow = lax.broadcasted_iota(jnp.int32, (16, D), 0)
        gblk = jnp.where(grow == 0, jnp.broadcast_to(gw_ref[...].astype(F32), (16, D)), 0.0)

        for br in range(2):
            (cp_wa, cp_wb)[br].wait()
            wt = w_s[br].astype(F32).T
            wt_s[br, 0:3 * D, :] = wt
            if br == 0:
                wt_s[br, 3 * D:3 * D + 16, :] = gblk
                cp_x.wait()
            for h in range(H):
                src = D + h * DH
                wkp_s[br * HP + h * DP: br * HP + (h + 1) * DP, :] = jnp.concatenate(
                    [wt_s[br, src:src + DH, :], zpad], axis=0).astype(BF16)
            xt = xt_s[...]
            if do_proj:
                tmp_s[0:D, :] = jnp.dot(wt_s[br, 0:D, :].astype(BF16), xt, preferred_element_type=F32) * QSCALE
                for h in range(H):
                    r0 = br * 2 * HP + h * DP
                    qvt_s[r0:r0 + DP, :] = jnp.concatenate([tmp_s[h * DH:(h + 1) * DH, :], zrow], axis=0).astype(BF16)
                n = D + 16 if br == 0 else D
                tmp_s[D:D + n, :] = jnp.dot(wt_s[br, 2 * D:2 * D + n, :].astype(BF16), xt, preferred_element_type=F32)
                for h in range(H):
                    r0 = br * 2 * HP + HP + h * DP
                    qvt_s[r0:r0 + DP, :] = jnp.concatenate([tmp_s[D + h * DH:D + (h + 1) * DH, :], onerow], axis=0).astype(BF16)
                if br == 0:
                    g_s[...] = jax.nn.sigmoid(tmp_s[2 * D:2 * D + 8, :])
                x = xt.T
                for grp in range(4):
                    kk = lax.dot_general(x, wkp_s[br * HP + grp * 128:br * HP + (grp + 1) * 128, :], NT, preferred_element_type=F32)
                    for j in range(4):
                        kh_s[br * H + grp * 4 + j] = kk[:, j * DP:(j + 1) * DP].astype(BF16)
        for br in range(2):
            (cp_woa, cp_wob)[br].wait()
            tmp_s[0:D, 0:D] = wo_s[br].astype(F32)
            wo_p = jnp.concatenate(
                [jnp.concatenate([tmp_s[h * DH:(h + 1) * DH, 0:D], zpad], axis=0) for h in range(H)], axis=0)
            wop_s[:, br * HP:(br + 1) * HP] = wo_p.T.astype(BF16)

        def rows(h):
            br = h // H
            hh = h % H
            return (br, pl.multiple_of(br * 2 * HP + hh * DP, DP), pl.multiple_of(br * 2 * HP + HP + hh * DP, DP),
                    pl.multiple_of(h * DP, DP))
        def scores(h, qi, c):
            qrow = rows(h)[1]
            qt = qvt_s[pl.ds(qrow, DP), qi * TQ:(qi + 1) * TQ]
            return jnp.dot(kh_s[h, c * CK:(c + 1) * CK, :], qt, preferred_element_type=F32)
        base = [(qi, c) for qi in range(NQ) for c in range(NC)]

        def body(it, carry):
            h0 = it * hpi
            steps = [(h0 + dh, qi, c) for dh in range(hpi) for (qi, c) in base]
            hn = jnp.minimum(h0 + hpi, NH - 1)
            allsteps = steps + [(hn, 0, 0)]
            s_next = sc_s[...]
            for i, (h, qi, c) in enumerate(steps):
                br, _, vrow, orow = rows(h)
                s = s_next
                s_next = scores(*allsteps[i + 1])
                if i + 1 == len(steps):
                    sc_s[...] = s_next
                cm = jnp.max(jnp.max(s.reshape(CK // 8, 8, TQ), axis=0), axis=0, keepdims=True)
                vt = qvt_s[pl.ds(vrow, DP), c * CK:(c + 1) * CK]
                if c == 0:
                    m = cm
                    p = jnp.exp2(s - m).astype(BF16)
                    acc = jnp.dot(vt, p, preferred_element_type=F32)
                else:
                    mn = jnp.maximum(m, cm)
                    alpha = jnp.exp2(m - mn)
                    p = jnp.exp2(s - mn).astype(BF16)
                    acc = acc * alpha + jnp.dot(vt, p, preferred_element_type=F32)
                    m = mn
                if c == NC - 1:
                    l = acc[DH:DH + 1, :]
                    g = g_s[0:1, qi * TQ:(qi + 1) * TQ]
                    gg = jnp.where(br == 0, g, 1.0 - g)
                    ot_s[pl.ds(orow, DP), qi * TQ:(qi + 1) * TQ] = (acc * (gg / l)).astype(BF16)
            return carry
        if do_attn:
            sc_s[...] = scores(0, 0, 0)
            lax.fori_loop(0, NH // hpi, body, 0)

        cps = []
        for oc in range(NOC):
            if do_out:
                outt = jnp.dot(wop_s[...], ot_s[:, oc * OC:(oc + 1) * OC], preferred_element_type=F32)
            else:
                outt = jnp.zeros((D, OC), F32)
            out_s[oc] = outt.astype(BF16)
            cp = pltpu.make_async_copy(out_s.at[oc], o_hbm.at[:, oc * OC:(oc + 1) * OC], sems.at[5 + oc])
            cp.start()
            cps.append(cp)
        for cp in cps:
            cp.wait()

    @jax.jit
    def f(A_x, A_wqkv, A_wo, B_x, B_wqkv, B_wo, gate_w):
        xt = A_x.reshape(S, D).T
        anyspec = pl.BlockSpec(memory_space=pl.ANY)
        out = pl.pallas_call(
            kernel,
            out_shape=jax.ShapeDtypeStruct((D, S), BF16),
            in_specs=[anyspec] * 5 + [pl.BlockSpec(memory_space=pltpu.VMEM)],
            out_specs=anyspec,
            scratch_shapes=[
                pltpu.VMEM((D, S), BF16),
                pltpu.VMEM((2, D, 3 * D), BF16),
                pltpu.VMEM((2, D, D), BF16),
                pltpu.VMEM((2, 3 * D + 16, D), F32),
                pltpu.VMEM((2 * HP, D), BF16),
                pltpu.VMEM((D, 2 * HP), BF16),
                pltpu.VMEM((2 * D + 16, S), F32),
                pltpu.VMEM((4 * HP, S), BF16),
                pltpu.VMEM((NH, S, DP), BF16),
                pltpu.VMEM((NH * DP, S), BF16),
                pltpu.VMEM((8, S), F32),
                pltpu.VMEM((CK, TQ), F32),
                pltpu.VMEM((NOC, D, OC), BF16),
                pltpu.SemaphoreType.DMA((5 + NOC,)),
            ],
            compiler_params=pltpu.CompilerParams(vmem_limit_bytes=100 * 2**20),
        )(xt, A_wqkv, A_wo, B_wqkv, B_wo, gate_w.reshape(1, D))
        return out.T.reshape(1, S, D)
    return f


pallas_gated_mix__mha_block__mha_block__prompt_kernel = _make()
```

```python
import math

import jax
import jax.numpy as jnp
from jax import lax
from jax.experimental import pallas as pl
from jax.experimental.pallas import tpu as pltpu

S, D, H, DH, DP = 2048, 448, 16, 28, 32
NH = 2 * H
HP = H * DP
QSCALE = (DH ** -0.5) * math.log2(math.e)
F32 = jnp.float32
BF16 = jnp.bfloat16

TQ = 1024
CK = 128
HPI = 2
OC = 512
XC = 1024
NQ = S // TQ
NC = S // CK
NOC = S // OC
NXC = S // XC


def _kernel(xt_hbm, wa_hbm, woa_hbm, wb_hbm, wob_hbm, gw_ref, o_hbm,
            xt_s, w_s, wo_s, wt_s, wot_s, wkt_s, wop_s, tmp_s, qvt_s, kh_s, ot_s,
            g_s, sc_s, out_s, sems):
    nt_dims = (((1,), (1,)), ((), ()))

    cp_wa0 = pltpu.make_async_copy(wa_hbm.at[:, 0:512], w_s.at[0, :, 0:512], sems.at[0])
    cp_x = [pltpu.make_async_copy(xt_hbm.at[:, j * XC:(j + 1) * XC],
                                  xt_s.at[:, j * XC:(j + 1) * XC], sems.at[5 + j])
            for j in range(NXC)]
    cp_wa1 = pltpu.make_async_copy(wa_hbm.at[:, 512:3 * D], w_s.at[0, :, 512:3 * D], sems.at[1])
    cp_wb = pltpu.make_async_copy(wb_hbm, w_s.at[1], sems.at[2])
    cp_woa = pltpu.make_async_copy(woa_hbm, wo_s.at[0], sems.at[3])
    cp_wob = pltpu.make_async_copy(wob_hbm, wo_s.at[1], sems.at[4])
    for cp in [cp_wa0] + cp_x + [cp_wa1, cp_wb, cp_woa, cp_wob]:
        cp.start()

    zrow = jnp.zeros((DP - DH, S), F32)
    prow = lax.broadcasted_iota(jnp.int32, (DP - DH, S), 0)
    onerow = jnp.where(prow == 0, 1.0, 0.0).astype(F32)
    grow = lax.broadcasted_iota(jnp.int32, (16, D), 0)
    gblk = jnp.where(grow == 0,
                     jnp.broadcast_to(gw_ref[...].astype(F32).reshape(1, D), (16, D)),
                     0.0).astype(BF16)

    def put_heads(src0, r0, pad):
        for h in range(H):
            qvt_s[r0 + h * DP:r0 + (h + 1) * DP, :] = jnp.concatenate(
                [tmp_s[src0 + h * DH:src0 + (h + 1) * DH, :], pad], axis=0).astype(BF16)

    cp_wa0.wait()
    cp_x[0].wait()
    wq = w_s[0, :, 0:512].astype(F32).T[0:D, :].astype(BF16)
    tmp_s[0:D, 0:XC] = jnp.dot(wq, xt_s[:, 0:XC], preferred_element_type=F32) * QSCALE
    for j in range(1, NXC):
        cp_x[j].wait()
    cp_wa1.wait()
    tmp_s[0:D, XC:S] = jnp.dot(wq, xt_s[:, XC:S], preferred_element_type=F32) * QSCALE
    wt_s[0] = w_s[0].astype(F32).T
    put_heads(0, 0, zrow)

    cp_wb.wait()
    cp_woa.wait()
    cp_wob.wait()
    xt = xt_s[...]
    wv = jnp.concatenate([wt_s[0, 2 * D:3 * D, :].astype(BF16), gblk], axis=0)
    tmp_s[D:2 * D + 16, :] = jnp.dot(wv, xt, preferred_element_type=F32)
    put_heads(D, HP, onerow)
    g_s[...] = jax.nn.sigmoid(tmp_s[2 * D:2 * D + 8, :])
    wt_s[1] = w_s[1].astype(F32).T
    for br in range(2):
        wkt_s[br * D:(br + 1) * D, :] = wt_s[br, D:2 * D, :].astype(BF16)

    x = xt.T
    zk = jnp.zeros((S, DP - DH), F32)
    kk = lax.dot_general(x, wkt_s[...], nt_dims, preferred_element_type=F32)
    for h in range(NH):
        kh_s[h] = jnp.concatenate([kk[:, h * DH:(h + 1) * DH], zk], axis=1).astype(BF16)
    for br in range(2):
        wot_s[br * D:(br + 1) * D, :] = wo_s[br].astype(F32)
    wop_s[...] = wot_s[...].T.astype(BF16)

    tmp_s[0:D, :] = jnp.dot(wt_s[1, 0:D, :].astype(BF16), xt, preferred_element_type=F32) * QSCALE
    put_heads(0, 2 * HP, zrow)
    tmp_s[D:2 * D, :] = jnp.dot(wt_s[1, 2 * D:3 * D, :].astype(BF16), xt, preferred_element_type=F32)
    put_heads(D, 3 * HP, onerow)

    def rows(h):
        br = h // H
        hh = h % H
        return (br,
                pl.multiple_of(br * 2 * HP + hh * DP, DP),
                pl.multiple_of(br * 2 * HP + HP + hh * DP, DP))

    def scores(h, qi, c):
        qt = qvt_s[pl.ds(rows(h)[1], DP), qi * TQ:(qi + 1) * TQ]
        return jnp.dot(kh_s[h, c * CK:(c + 1) * CK, :], qt, preferred_element_type=F32)

    base = [(qi, c) for qi in range(NQ) for c in range(NC)]

    def body(it, carry):
        h0 = it * HPI
        steps = [(h0 + dh, qi, c) for dh in range(HPI) for (qi, c) in base]
        hn = jnp.minimum(h0 + HPI, NH - 1)
        allsteps = steps + [(hn, 0, 0)]
        s_next = sc_s[...]
        staged = {}
        m = acc = None
        for i, (h, qi, c) in enumerate(steps):
            br, _, vrow = rows(h)
            s = s_next
            s_next = scores(*allsteps[i + 1])
            if i + 1 == len(steps):
                sc_s[...] = s_next
            cm = jnp.max(jnp.max(s.reshape(CK // 8, 8, TQ), axis=0), axis=0, keepdims=True)
            vt = qvt_s[pl.ds(vrow, DP), c * CK:(c + 1) * CK]
            if c == 0:
                m = cm
                p = jnp.exp2(s - m).astype(BF16)
                acc = jnp.dot(vt, p, preferred_element_type=F32)
            else:
                mn = jnp.maximum(m, cm)
                alpha = jnp.exp2(m - mn)
                p = jnp.exp2(s - mn).astype(BF16)
                acc = acc * alpha + jnp.dot(vt, p, preferred_element_type=F32)
                m = mn
            if c == NC - 1:
                l = acc[DH:DH + 1, :]
                g = g_s[0:1, qi * TQ:(qi + 1) * TQ]
                gg = jnp.where(br == 0, g, 1.0 - g)
                staged.setdefault(qi, []).append((acc * (gg / l))[0:DH, :])
                if len(staged[qi]) == HPI:
                    r0 = pl.multiple_of(it * (HPI * DH), 8)
                    ot_s[pl.ds(r0, HPI * DH), qi * TQ:(qi + 1) * TQ] = jnp.concatenate(
                        staged[qi], axis=0)
        return carry

    sc_s[...] = scores(0, 0, 0)
    lax.fori_loop(0, NH // HPI, body, 0)

    cps = []
    for oc in range(NOC):
        outt = jnp.dot(wop_s[...], ot_s[:, oc * OC:(oc + 1) * OC].astype(BF16),
                       preferred_element_type=F32)
        out_s[oc] = outt.astype(BF16)
        cp = pltpu.make_async_copy(out_s.at[oc], o_hbm.at[:, oc * OC:(oc + 1) * OC],
                                   sems.at[5 + NXC + oc])
        cp.start()
        cps.append(cp)
    for cp in cps:
        cp.wait()


@jax.jit
def pallas_gated_mix__mha_block__mha_block__prompt_kernel(
    A_x: jax.Array,
    A_wqkv: jax.Array,
    A_wo: jax.Array,
    B_x: jax.Array,
    B_wqkv: jax.Array,
    B_wo: jax.Array,
    gate_w: jax.Array,
):
    del B_x
    xt = A_x.reshape(S, D).T
    anyspec = pl.BlockSpec(memory_space=pl.ANY)
    out_t = pl.pallas_call(
        _kernel,
        out_shape=jax.ShapeDtypeStruct((D, S), BF16),
        in_specs=[anyspec] * 5 + [pl.BlockSpec(memory_space=pltpu.VMEM)],
        out_specs=anyspec,
        scratch_shapes=[
            pltpu.VMEM((D, S), BF16),
            pltpu.VMEM((2, D, 3 * D), BF16),
            pltpu.VMEM((2, D, D), BF16),
            pltpu.VMEM((2, 3 * D, D), F32),
            pltpu.VMEM((2 * D, D), F32),
            pltpu.VMEM((2 * D, D), BF16),
            pltpu.VMEM((D, 2 * D), BF16),
            pltpu.VMEM((2 * D + 16, S), F32),
            pltpu.VMEM((4 * HP, S), BF16),
            pltpu.VMEM((NH, S, DP), BF16),
            pltpu.VMEM((NH * DH, S), F32),
            pltpu.VMEM((8, S), F32),
            pltpu.VMEM((CK, TQ), F32),
            pltpu.VMEM((NOC, D, OC), BF16),
            pltpu.SemaphoreType.DMA((5 + NXC + NOC,)),
        ],
        compiler_params=pltpu.CompilerParams(vmem_limit_bytes=100 * 2**20),
    )(xt, A_wqkv, A_wo, B_wqkv, B_wo, gate_w)
    return out_t.T.reshape(1, S, D)
```
